```python
import os as _os
_os.environ.setdefault("JAX_PLATFORMS", "cpu")
import jax
import jax.numpy as jnp

def _softmax(x, axis=-1):
    return jax.nn.softmax(x, axis=axis)
def _gelu(x):
    return jax.nn.gelu(x, approximate=True)
def _silu(x):
    return jax.nn.silu(x)
def _sigmoid(x):
    return jax.nn.sigmoid(x)
def _layernorm(x, axis=-1, eps=1e-5):
    m = jnp.mean(x, axis=axis, keepdims=True)
    v = jnp.var(x, axis=axis, keepdims=True)
    return (x - m) / jnp.sqrt(v + eps)
def _scatter_add(tgt, idx, src, axis=0):
    return tgt.at[idx].add(src)
def _segment_sum(src, seg, n):
    return jax.ops.segment_sum(src, seg, n)
class _Rng:
    def __init__(self, key):
        self._k = key
    def _next(self):
        self._k, sub = jax.random.split(self._k)
        return sub
    def normal(self, shape):
        return jax.random.normal(self._next(), shape, dtype=jnp.bfloat16)
    def randint(self, lo, hi, shape):
        return jax.random.randint(self._next(), shape, lo, hi, dtype=jnp.int32)
    def uniform(self, shape, lo=0.0, hi=1.0):
        return jax.random.uniform(self._next(), shape, jnp.bfloat16, lo, hi)
    def permutation(self, n):
        return jax.random.permutation(self._next(), n)


kernel_name = 'standalone__dcn_v2_cross__recsys'

def setup_inputs():
    _rng = _Rng(jax.random.key(int.from_bytes(__import__("os").urandom(4), "little")))
    _w = (lambda a: (lambda t: t.astype(jnp.bfloat16) if jnp.issubdtype(t.dtype, jnp.floating) else t)(jnp.asarray(a)))
    B, F, D, L = 4096, 26, 128, 6
    Din = min(F * D, 1024)
    return {
        "x0": _w((lambda *s: _rng.normal(s) * 0.05)(B, Din)),
        "ws": _w((lambda *s: _rng.normal(s) * 0.05)(L, Din, Din)),
        "bs": _w((lambda *s: _rng.normal(s) * 0.05)(L, Din)),
    }

def reference(x0, ws, bs):
    x = x0
    for l in range(ws.shape[0]):
        x = x0 * (x @ ws[l] + bs[l]) + x
    return x
```

```python
import jax
import jax.numpy as jnp
import jax.experimental.pallas as pl
import jax.experimental.pallas.tpu as pltpu


@jax.jit
def pallas_standalone__dcn_v2_cross__recsys_kernel(
    x0: jax.Array,
    ws: jax.Array,
    bs: jax.Array,
):
    B, D = x0.shape
    L = ws.shape[0]
    bm = min(256, B)
    h = D // 2
    f32 = jnp.float32

    def kern(x0_ref, w0a_ref, ws_hbm, bs_ref, o_ref, w_vmem, sems):
        i = pl.program_id(0)
        copies = [
            pltpu.make_async_copy(ws_hbm.at[l], w_vmem.at[l], sems.at[l])
            for l in range(L)
        ]

        def run(first):
            x = x0_ref[...]
            for l in range(L):
                if first and l == 0:
                    ya = jnp.dot(x, w0a_ref[0], preferred_element_type=f32)
                    copies[0].wait()
                    yb = jnp.dot(x, w_vmem[0, :, h:], preferred_element_type=f32)
                    y = jnp.concatenate([ya, yb], axis=1)
                else:
                    if first:
                        copies[l].wait()
                    y = jnp.dot(x, w_vmem[l], preferred_element_type=f32)
                y = y + bs_ref[l:l + 1, :].astype(f32)
                x = (x0_ref[...].astype(f32) * y + x.astype(f32)).astype(x.dtype)
            o_ref[...] = x

        @pl.when(i == 0)
        def _():
            for c in copies:
                c.start()
            run(True)

        @pl.when(i > 0)
        def _():
            run(False)

    return pl.pallas_call(
        kern,
        grid=(pl.cdiv(B, bm),),
        in_specs=[
            pl.BlockSpec((bm, D), lambda i: (i, 0)),
            pl.BlockSpec((1, D, h), lambda i: (0, 0, 0), pipeline_mode=pl.Buffered(1)),
            pl.BlockSpec(memory_space=pl.ANY),
            pl.BlockSpec((L, D), lambda i: (0, 0)),
        ],
        out_specs=pl.BlockSpec((bm, D), lambda i: (i, 0)),
        out_shape=jax.ShapeDtypeStruct((B, D), x0.dtype),
        scratch_shapes=[
            pltpu.VMEM((L, D, D), ws.dtype),
            pltpu.SemaphoreType.DMA((L,)),
        ],
        compiler_params=pltpu.CompilerParams(
            dimension_semantics=("arbitrary",), vmem_limit_bytes=64 * 2**20
        ),
    )(x0, ws, ws, bs)
```

```python
import jax
import jax.numpy as jnp
import jax.experimental.pallas as pl
import jax.experimental.pallas.tpu as pltpu


@jax.jit
def pallas_standalone__dcn_v2_cross__recsys_kernel(
    x0: jax.Array,
    ws: jax.Array,
    bs: jax.Array,
):
    B, D = x0.shape
    L = ws.shape[0]
    bm = min(256, B)
    f32 = jnp.float32

    def kern(x0_ref, ws_hbm, bs_ref, o_ref, w_vmem, b_vmem, sems):
        i = pl.program_id(0)

        def w_copy(l):
            return pltpu.make_async_copy(ws_hbm.at[l], w_vmem.at[l], sems.at[l])

        def layer(x, w, b):
            y = jnp.dot(x, w, preferred_element_type=f32) + b
            return (x0_ref[...].astype(f32) * y + x.astype(f32)).astype(x.dtype)

        @pl.when(i == 0)
        def _():
            for l in range(L):
                w_copy(l).start()
            b_vmem[...] = bs_ref[...].astype(f32)
            o_ref[...] = x0_ref[...]

            def body(l, carry):
                w_copy(l).wait()
                o_ref[...] = layer(o_ref[...], w_vmem[l], b_vmem[pl.ds(l, 1), :])
                return carry

            jax.lax.fori_loop(0, L, body, 0)

        @pl.when(i > 0)
        def _():
            x = x0_ref[...]
            for l in range(L):
                x = layer(x, w_vmem[l], b_vmem[l:l + 1, :])
            o_ref[...] = x

    return pl.pallas_call(
        kern,
        grid=(pl.cdiv(B, bm),),
        in_specs=[
            pl.BlockSpec((bm, D), lambda i: (i, 0)),
            pl.BlockSpec(memory_space=pl.ANY),
            pl.BlockSpec((L, D), lambda i: (0, 0)),
        ],
        out_specs=pl.BlockSpec((bm, D), lambda i: (i, 0)),
        out_shape=jax.ShapeDtypeStruct((B, D), x0.dtype),
        scratch_shapes=[
            pltpu.VMEM((L, D, D), ws.dtype),
            pltpu.VMEM((L, D), f32),
            pltpu.SemaphoreType.DMA((L,)),
        ],
        compiler_params=pltpu.CompilerParams(
            dimension_semantics=("arbitrary",), vmem_limit_bytes=100 * 2**20
        ),
    )(x0, ws, bs)
```
